```python
import os as _os
_os.environ.setdefault("JAX_PLATFORMS", "cpu")
import jax
import jax.numpy as jnp

def _softmax(x, axis=-1):
    return jax.nn.softmax(x, axis=axis)
def _gelu(x):
    return jax.nn.gelu(x, approximate=True)
def _silu(x):
    return jax.nn.silu(x)
def _sigmoid(x):
    return jax.nn.sigmoid(x)
def _layernorm(x, axis=-1, eps=1e-5):
    m = jnp.mean(x, axis=axis, keepdims=True)
    v = jnp.var(x, axis=axis, keepdims=True)
    return (x - m) / jnp.sqrt(v + eps)
def _scatter_add(tgt, idx, src, axis=0):
    return tgt.at[idx].add(src)
def _segment_sum(src, seg, n):
    return jax.ops.segment_sum(src, seg, n)
class _Rng:
    def __init__(self, key):
        self._k = key
    def _next(self):
        self._k, sub = jax.random.split(self._k)
        return sub
    def normal(self, shape):
        return jax.random.normal(self._next(), shape, dtype=jnp.bfloat16)
    def randint(self, lo, hi, shape):
        return jax.random.randint(self._next(), shape, lo, hi, dtype=jnp.int32)
    def uniform(self, shape, lo=0.0, hi=1.0):
        return jax.random.uniform(self._next(), shape, jnp.bfloat16, lo, hi)
    def permutation(self, n):
        return jax.random.permutation(self._next(), n)


kernel_name = 'interleave_layers__sliding_block_cached__mixer_channel_mlp__decode'

def setup_inputs():
    _rng = _Rng(jax.random.key(int.from_bytes(__import__("os").urandom(4), "little")))
    _w = (lambda a: (lambda t: t.astype(jnp.bfloat16) if jnp.issubdtype(t.dtype, jnp.floating) else t)(jnp.asarray(a)))
    def _A_setup():
        B, Sq, D = 8, 1, 1024
        Hq, Hkv, Sk, Dh = 32, 4, 4096, 128
        assert Hq % Hkv == 0, (Hq, Hkv)
        return {
            "x": _w((lambda *s: _rng.normal(s) * 0.05)(B, Sq, D)),
            "k_cache": _w((lambda *s: _rng.normal(s) * 1.6)(B, Hkv, Sk, Dh)),
            "v_cache": _w((lambda *s: _rng.normal(s) * 0.8)(B, Hkv, Sk, Dh)),
            "wq": _w((lambda *s: _rng.normal(s) * 1.6)(D, Hq * Dh) * (D ** -0.5)),
            "wo": _w((lambda *s: _rng.normal(s) * 0.8)(Hq * Dh, D) * ((Hq * Dh) ** -0.5)),
        }
    _A_in = _A_setup()

    def _B_setup():
        B, S, D, F = 8, 1, 1024, 3584
        return {
            "x": _w((lambda *s: _rng.normal(s) * 0.05)(B, S, D)),
            "w1": _w((lambda *s: _rng.normal(s) * 0.4)(D, F) * (D ** -0.5)),
            "b1": _w((lambda *s: _rng.normal(s) * 0.4)(F)),
            "w2": _w((lambda *s: _rng.normal(s) * 0.4)(F, D) * (F ** -0.5)),
            "b2": _w((lambda *s: _rng.normal(s) * 0.1)(D)),
        }
    _B_in = _B_setup()

    return {
        "A_x": _A_in["x"],
        "A_k_cache": _A_in["k_cache"],
        "A_v_cache": _A_in["v_cache"],
        "A_wq": _A_in["wq"],
        "A_wo": _A_in["wo"],
        "B_x": _B_in["x"],
        "B_w1": _B_in["w1"],
        "B_b1": _B_in["b1"],
        "B_w2": _B_in["w2"],
        "B_b2": _B_in["b2"],
    }

def reference(A_x, A_k_cache, A_v_cache, A_wq, A_wo, B_x, B_w1, B_b1, B_w2, B_b2):
    def _A_ref(x, k_cache, v_cache, wq, wo):
        B, Sq, D = x.shape
        Hq, Dh = 32, 128
        Hkv, Sk = k_cache.shape[1], k_cache.shape[2]
        W = min(4096, max(256, Sk // 4))
        rep = Hq // Hkv
        q = (lambda x, *d: x.transpose(*d))((x @ wq).reshape(B, Sq, Hq, Dh), 0, 2, 1, 3)
        k = jnp.repeat(k_cache[:, :, Sk - W:, :], rep, axis=1)
        v = jnp.repeat(v_cache[:, :, Sk - W:, :], rep, axis=1)
        scores = jnp.einsum("bhqd,bhkd->bhqk", q, k) * (Dh ** -0.5)
        p = _softmax(scores, axis=-1)
        o = jnp.einsum("bhqk,bhkd->bhqd", p, v)
        return (lambda x, *d: x.transpose(*d))(o, 0, 2, 1, 3).reshape(B, Sq, Hq * Dh) @ wo

    def _B_ref(x, w1, b1, w2, b2):
        y = _layernorm(x, axis=-1)
        h = _gelu(jnp.einsum("bsd,df->bsf", y, w1) + b1)
        return jnp.einsum("bsf,fd->bsd", h, w2) + b2

    x = A_x
    x = x + _A_ref(_layernorm(x, axis=-1), A_k_cache, A_v_cache, A_wq, A_wo)
    x = x + _B_ref(_layernorm(x, axis=-1), B_w1, B_b1, B_w2, B_b2)
    x = x + _A_ref(_layernorm(x, axis=-1), A_k_cache, A_v_cache, A_wq, A_wo)
    x = x + _B_ref(_layernorm(x, axis=-1), B_w1, B_b1, B_w2, B_b2)
    return x
```

```python
import jax
import jax.numpy as jnp
import jax.experimental.pallas as pl
import jax.experimental.pallas.tpu as pltpu

B, D = 8, 1024
HQ, HKV, SK, DH = 32, 4, 4096, 128
W = min(4096, max(256, SK // 4))
REP = HQ // HKV
F = 3584
EPS = 1e-5
PAD = 128
NBG = B * HKV

f32 = jnp.float32
bf16 = jnp.bfloat16


def _ln(x):
    m = jnp.mean(x, axis=-1, keepdims=True)
    xc = x - m
    v = jnp.mean(xc * xc, axis=-1, keepdims=True)
    return xc * jax.lax.rsqrt(v + EPS)


def _gelu(x):
    c = 0.7978845608028654
    return 0.5 * x * (1.0 + jnp.tanh(c * (x + 0.044715 * (x * x * x))))


def _kernel(x_hbm, k_hbm, v_hbm, wq_hbm, wo_hbm, w1_hbm, b1_hbm, w2_hbm, b2_hbm,
            o_ref,
            x_buf, b1_buf, b2_buf, wq_buf, k_buf, v_buf, wo_buf, w1_buf, w2_buf,
            q_scr, o_scr, sems):
    cp = pltpu.make_async_copy
    c_x = cp(x_hbm, x_buf, sems.at[0])
    c_b1 = cp(b1_hbm, b1_buf, sems.at[1])
    c_b2 = cp(b2_hbm, b2_buf, sems.at[2])
    c_wq = cp(wq_hbm, wq_buf.at[:, pl.ds(0, HQ * DH)], sems.at[3])
    c_k = [cp(k_hbm.at[b, :, pl.ds(SK - W, W), :], k_buf.at[b], sems.at[4 + b]) for b in range(B)]
    c_v = [cp(v_hbm.at[b, :, pl.ds(SK - W, W), :], v_buf.at[b], sems.at[12 + b]) for b in range(B)]
    c_wo = cp(wo_hbm, wo_buf.at[:, pl.ds(0, D)], sems.at[20])
    c_w1 = cp(w1_hbm, w1_buf.at[:, pl.ds(0, F)], sems.at[21])
    c_w2 = cp(w2_hbm, w2_buf.at[:, pl.ds(0, D)], sems.at[22])

    c_x.start()
    c_wq.start()
    for c in c_k:
        c.start()
    for c in c_v:
        c.start()
    c_wo.start()
    c_b1.start()
    c_b2.start()
    c_w1.start()
    c_w2.start()

    def attn(x, first):
        xn = _ln(x).astype(bf16)
        if first:
            c_wq.wait()
        q = jnp.dot(xn, wq_buf[:, 0:HQ * DH], preferred_element_type=f32) * (DH ** -0.5)
        for h in range(HQ):
            q_scr[h * B:(h + 1) * B, :] = q[:, h * DH:(h + 1) * DH]
        for b in range(B):
            if first:
                c_k[b].wait()
        ps = []
        for b in range(B):
            for g in range(HKV):
                qg = q_scr[pl.ds(g * REP * B + b, REP, stride=B), :].astype(bf16)
                s = jax.lax.dot_general(qg, k_buf[b, g], (((1,), (1,)), ((), ())),
                                        preferred_element_type=f32)
                m = jnp.max(s, axis=-1, keepdims=True)
                p = jnp.exp(s - m)
                l = jnp.sum(p, axis=-1, keepdims=True)
                ps.append((p.astype(bf16), l))
        for b in range(B):
            if first:
                c_v[b].wait()
            for g in range(HKV):
                p, l = ps[b * HKV + g]
                o = jnp.dot(p, v_buf[b, g], preferred_element_type=f32) / l
                o_scr[pl.ds(g * REP * B + b, REP, stride=B), :] = o
        oall = jnp.concatenate([o_scr[h * B:(h + 1) * B, :] for h in range(HQ)], axis=1).astype(bf16)
        if first:
            c_wo.wait()
        return x + jnp.dot(oall, wo_buf[:, 0:D], preferred_element_type=f32)

    def mlp(x, first):
        y = _ln(_ln(x)).astype(bf16)
        if first:
            c_b1.wait()
            c_b2.wait()
            c_w1.wait()
        b1 = b1_buf[...].reshape(1, F).astype(f32)
        b2 = b2_buf[...].reshape(1, D).astype(f32)
        h = _gelu(jnp.dot(y, w1_buf[:, 0:F], preferred_element_type=f32) + b1).astype(bf16)
        if first:
            c_w2.wait()
        return x + jnp.dot(h, w2_buf[:, 0:D], preferred_element_type=f32) + b2

    c_x.wait()
    x = x_buf[...].astype(f32)
    x = attn(x, True)
    x = mlp(x, True)
    x = attn(x, False)
    x = mlp(x, False)
    o_ref[...] = x.astype(o_ref.dtype)


@jax.jit
def pallas_interleave_layers__sliding_block_cached__mixer_channel_mlp__decode_kernel(
    A_x, A_k_cache, A_v_cache, A_wq, A_wo, B_x, B_w1, B_b1, B_w2, B_b2,
):
    del B_x
    any_spec = pl.BlockSpec(memory_space=pl.ANY)
    out = pl.pallas_call(
        _kernel,
        out_shape=jax.ShapeDtypeStruct((B, D), A_x.dtype),
        in_specs=[any_spec] * 9,
        out_specs=pl.BlockSpec(memory_space=pltpu.VMEM),
        scratch_shapes=[
            pltpu.VMEM((B, D), bf16),
            pltpu.VMEM((F,), bf16),
            pltpu.VMEM((D,), bf16),
            pltpu.VMEM((D, HQ * DH + PAD), bf16),
            pltpu.VMEM((B, HKV, W, DH), bf16),
            pltpu.VMEM((B, HKV, W, DH), bf16),
            pltpu.VMEM((HQ * DH, D + PAD), bf16),
            pltpu.VMEM((D, F + PAD), bf16),
            pltpu.VMEM((F, D + PAD), bf16),
            pltpu.VMEM((HQ * B, DH), f32),
            pltpu.VMEM((HQ * B, DH), f32),
            pltpu.SemaphoreType.DMA((23,)),
        ],
        compiler_params=pltpu.CompilerParams(vmem_limit_bytes=100 * 1024 * 1024),
    )(A_x.reshape(B, D), A_k_cache, A_v_cache, A_wq, A_wo, B_w1, B_b1, B_w2, B_b2)
    return out.reshape(B, 1, D)
```

```python
import jax
import jax.numpy as jnp
import jax.experimental.pallas as pl
import jax.experimental.pallas.tpu as pltpu

B, D = 8, 1024
HQ, HKV, SK, DH = 32, 4, 4096, 128
W = min(4096, max(256, SK // 4))
REP = HQ // HKV
F = 3584
EPS = 1e-5
PAD = 128
NQ = HQ * DH
SB = W // 128
SCALE = DH ** -0.5

W2_PIECES = (
    (0, 1792, 0, 896), (1792, 1280, 0, 768), (3072, 512, 0, 768),
    (1792, 1792, 768, 128),
    (0, 3072, 896, 128), (3072, 512, 896, 128),
)
W1_HEAD = (512, 1024)
QCH, OCH, HCH = 512, 128, 512
LOOKAHEAD = 4

SEM_X, SEM_WQ, SEM_WO, SEM_B1, SEM_B2, SEM_W1 = range(6)
SEM_K = 6
SEM_V = SEM_K + B
SEM_W2 = SEM_V + B
N_SEMS = SEM_W2 + len(W2_PIECES)

f32 = jnp.float32
bf16 = jnp.bfloat16


def _dot(a, b):
    return jnp.dot(a, b, preferred_element_type=f32)


def _ln_stats(x):
    m = jnp.mean(x, axis=-1, keepdims=True)
    xc = x - m
    v = jnp.mean(xc * xc, axis=-1, keepdims=True)
    return m, jax.lax.rsqrt(v + EPS)


def _ln(x):
    m, rs = _ln_stats(x)
    return (x - m) * rs


def _gelu(x):
    c = 0.7978845608028654
    return 0.5 * x * (1.0 + jnp.tanh(c * (x + 0.044715 * (x * x * x))))


def _body(x_hbm, k_hbm, v_hbm, wq_hbm, wo_hbm, w1_hbm, b1_hbm, w2_hbm, b2_hbm,
          o_ref,
          x_buf, b1_buf, b2_buf, wq_buf, k_buf, kt_buf, v_buf, wo_buf, w1_buf, w2_buf,
          q_scr, o_scr, qacc_scr, csq_scr, x1_scr, hh_scr, sems):
    cp = pltpu.make_async_copy

    def cp_k(b):
        return cp(k_hbm.at[b, :, pl.ds(SK - W, W), :], k_buf.at[b], sems.at[SEM_K + b])

    def cp_v(b):
        return cp(v_hbm.at[b, :, pl.ds(SK - W, W), :], v_buf.at[b], sems.at[SEM_V + b])

    c_x = cp(x_hbm, x_buf, sems.at[SEM_X])
    c_wq = cp(wq_hbm, wq_buf.at[:, pl.ds(0, NQ)], sems.at[SEM_WQ])
    c_wo = cp(wo_hbm, wo_buf.at[:, pl.ds(0, D)], sems.at[SEM_WO])
    c_b1 = cp(b1_hbm, b1_buf, sems.at[SEM_B1])
    c_b2 = cp(b2_hbm, b2_buf, sems.at[SEM_B2])
    c_w1 = cp(w1_hbm, w1_buf.at[:, pl.ds(0, F)], sems.at[SEM_W1])
    c_w2 = [cp(w2_hbm.at[pl.ds(r0, nr), pl.ds(c0, nc)],
               w2_buf.at[pl.ds(r0, nr), pl.ds(c0, nc)], sems.at[SEM_W2 + i])
            for i, (r0, nr, c0, nc) in enumerate(W2_PIECES)]

    c_wq.start()
    c_x.start()
    for b in range(B):
        cp_k(b).start()
        cp_v(b).start()
    c_wo.start()
    c_b1.start()
    c_b2.start()
    c_w1.start()
    for c in c_w2:
        c.start()

    ones8 = jnp.ones((B, D), f32)

    def attn_qk(b, g):
        qg = q_scr[pl.ds(g * REP * B + b, REP, stride=B), :].astype(bf16)
        s = jnp.concatenate([_dot(qg, kt_buf[b * HKV + g, j]) for j in range(SB)], axis=1)
        m = jnp.max(s, axis=-1, keepdims=True)
        p = jnp.exp(s - m)
        l = jnp.sum(p, axis=-1, keepdims=True)
        return p.astype(bf16), l

    def attn_pv(b, g, p_and_l):
        p, l = p_and_l
        o = _dot(p, v_buf[b, g]) / l
        o_scr[pl.ds(g * REP * B + b, REP, stride=B), :] = o

    def attn_pairs(pairs, la):
        pend = []
        for i, (b, g) in enumerate(pairs):
            pend.append(attn_qk(b, g))
            if i >= la:
                attn_pv(*pairs[i - la], pend[i - la])
        for i in range(max(len(pairs) - la, 0), len(pairs)):
            attn_pv(*pairs[i], pend[i])

    def get_o():
        return jnp.concatenate([o_scr[h * B:(h + 1) * B, :] for h in range(HQ)],
                               axis=1).astype(bf16)

    c_x.wait()
    c_wq.wait()
    x0 = x_buf[...].astype(f32)
    lhs_q = jnp.concatenate([_ln(x0), ones8], axis=0).astype(bf16)

    def l1_q(c, carry):
        c0 = pl.multiple_of(c * QCH, QCH)
        qq = _dot(lhs_q, wq_buf[:, pl.ds(c0, QCH)])
        csq_scr[:, pl.ds(c0, QCH)] = qq[B:2 * B]
        for h in range(QCH // DH):
            r0 = pl.multiple_of(c * (QCH // DH * B) + h * B, B)
            q_scr[pl.ds(r0, B), :] = qq[0:B, h * DH:(h + 1) * DH] * SCALE
        return carry

    jax.lax.fori_loop(0, NQ // QCH, l1_q, 0)

    def l1_attn(b, carry):
        cp_k(b).wait()
        cp_v(b).wait()
        for g in range(HKV):
            for t in range(SB):
                kt_buf[b * HKV + g, t] = k_buf[b, g, t * 128:(t + 1) * 128, :].T
        attn_pairs([(b, g) for g in range(HKV)], HKV)
        return carry

    jax.lax.fori_loop(0, B, l1_attn, 0)

    c_wo.wait()
    o_all = get_o()

    def l1_o(c, carry):
        c0 = pl.multiple_of(c * OCH, OCH)
        x1_scr[:, pl.ds(c0, OCH)] = _dot(o_all, wo_buf[:, pl.ds(c0, OCH)])
        return carry

    jax.lax.fori_loop(0, D // OCH, l1_o, 0)
    x1 = x0 + x1_scr[...]
    lhs_h = jnp.concatenate([_ln(_ln(x1)), ones8], axis=0).astype(bf16)
    c_b1.wait()
    c_b2.wait()
    c_w1.wait()
    b1 = b1_buf[...].reshape(1, F).astype(f32)
    b2 = b2_buf[...].reshape(1, D).astype(f32)

    def l1_h(c, carry):
        c0 = pl.multiple_of(c * HCH, HCH)
        hh_scr[:, pl.ds(c0, HCH)] = _dot(lhs_h, w1_buf[:, pl.ds(c0, HCH)])
        return carry

    jax.lax.fori_loop(0, F // HCH, l1_h, 0)
    h = _gelu(hh_scr[0:B, :] + b1).astype(bf16)
    x1b = x1 + b2

    nblk = D // 128
    acc = [x1b[:, j * 128:(j + 1) * 128] for j in range(nblk)]
    left = [F] * nblk
    x2_parts = [None] * nblk
    qacc = None
    shift = None
    for (r0, nr, c0, nc), c in zip(W2_PIECES, c_w2):
        c.wait()
        j0, j1 = c0 // 128, (c0 + nc) // 128
        d = (jnp.concatenate(acc[j0:j1], axis=1)
             + _dot(h[:, r0:r0 + nr], w2_buf[r0:r0 + nr, c0:c0 + nc]))
        done = []
        for j in range(j0, j1):
            acc[j] = d[:, (j - j0) * 128:(j - j0 + 1) * 128]
            left[j] -= nr
            if left[j] == 0:
                done.append(j)
        if done:
            assert done == list(range(done[0], done[-1] + 1))
            xr = jnp.concatenate([acc[j] for j in done], axis=1).astype(bf16)
            for j in done:
                x2_parts[j] = xr[:, (j - done[0]) * 128:(j - done[0] + 1) * 128].astype(f32)
            part = _dot(xr, wq_buf[done[0] * 128:(done[-1] + 1) * 128, 0:NQ])
            qacc = part if qacc is None else qacc_scr[...] + part
            if any(left):
                qacc_scr[...] = qacc
                shift = jnp.mean(
                    jnp.concatenate([p for p in x2_parts if p is not None], axis=1),
                    axis=-1, keepdims=True)
    assert not any(left)
    x2 = jnp.concatenate(x2_parts, axis=1)

    xc = x2 - shift
    d1 = jnp.mean(xc, axis=-1, keepdims=True)
    d2 = jnp.mean(xc * xc, axis=-1, keepdims=True)
    m = shift + d1
    rs = jax.lax.rsqrt(jnp.maximum(d2 - d1 * d1, 0.0) + EPS)
    q = (qacc - m * csq_scr[...]) * (rs * SCALE)
    for hd in range(HQ):
        q_scr[hd * B:(hd + 1) * B, :] = q[:, hd * DH:(hd + 1) * DH]
    attn_pairs([(b, g) for g in range(HKV) for b in range(B)], LOOKAHEAD)
    x3r = (x2 + _dot(get_o(), wo_buf[:, 0:D])).astype(bf16)
    x3 = x3r.astype(f32)
    hk, hn = W1_HEAD
    h_a = _dot(x3r[:, 0:hk], w1_buf[0:hk, 0:hn])
    h_a = _dot(x3r[:, hk:D], w1_buf[hk:D, 0:hn]) + h_a
    hraw = jnp.concatenate([h_a, _dot(x3r, w1_buf[:, hn:F])], axis=1)
    m1, rs1 = _ln_stats(x3)
    m2, rs2 = _ln_stats((x3 - m1) * rs1)
    a = rs1 * rs2
    c = (m1 * rs1 + m2) * rs2
    h = _gelu(hraw * a - hh_scr[B:2 * B, :] * c + b1).astype(bf16)
    out = x3 + b2 + _dot(h, w2_buf[:, 0:D])
    o_ref[...] = out.astype(o_ref.dtype)


def _kernel(*refs):
    pl.run_scoped(lambda sems: _body(*refs, sems), pltpu.SemaphoreType.DMA((N_SEMS,)))


@jax.jit
def pallas_interleave_layers__sliding_block_cached__mixer_channel_mlp__decode_kernel(
    A_x: jax.Array,
    A_k_cache: jax.Array,
    A_v_cache: jax.Array,
    A_wq: jax.Array,
    A_wo: jax.Array,
    B_x: jax.Array,
    B_w1: jax.Array,
    B_b1: jax.Array,
    B_w2: jax.Array,
    B_b2: jax.Array,
):
    del B_x
    any_spec = pl.BlockSpec(memory_space=pl.ANY)
    out = pl.pallas_call(
        _kernel,
        out_shape=jax.ShapeDtypeStruct((B, D), A_x.dtype),
        in_specs=[any_spec] * 9,
        out_specs=pl.BlockSpec(memory_space=pltpu.VMEM),
        scratch_shapes=[
            pltpu.VMEM((B, D), bf16),
            pltpu.VMEM((F,), bf16),
            pltpu.VMEM((D,), bf16),
            pltpu.VMEM((D, NQ + PAD), bf16),
            pltpu.VMEM((B, HKV, W, DH), bf16),
            pltpu.VMEM((B * HKV, SB, DH, 128), bf16),
            pltpu.VMEM((B, HKV, W, DH), bf16),
            pltpu.VMEM((NQ, D + PAD), bf16),
            pltpu.VMEM((D, F + PAD), bf16),
            pltpu.VMEM((F, D + PAD), bf16),
            pltpu.VMEM((HQ * B, DH), f32),
            pltpu.VMEM((HQ * B, DH), f32),
            pltpu.VMEM((B, NQ), f32),
            pltpu.VMEM((B, NQ), f32),
            pltpu.VMEM((B, D), f32),
            pltpu.VMEM((2 * B, F), f32),
        ],
        compiler_params=pltpu.CompilerParams(vmem_limit_bytes=100 * 1024 * 1024),
    )(A_x.reshape(B, D), A_k_cache, A_v_cache, A_wq, A_wo, B_w1, B_b1, B_w2, B_b2)
    return out.reshape(B, 1, D)
```
